```python
import jax
import jax.numpy as jnp

def _softmax(x, axis=-1):
    return jax.nn.softmax(x, axis=axis)

def _gelu(x):
    return jax.nn.gelu(x, approximate=True)

def _silu(x):
    return jax.nn.silu(x)

def _sigmoid(x):
    return jax.nn.sigmoid(x)

def _layernorm(x, axis=-1, eps=1e-05):
    m = jnp.mean(x, axis=axis, keepdims=True)
    v = jnp.var(x, axis=axis, keepdims=True)
    return (x - m) / jnp.sqrt(v + eps)

def _scatter_add(tgt, idx, src, axis=0):
    return tgt.at[idx].add(src)

def _segment_sum(src, seg, n):
    return jax.ops.segment_sum(src, seg, n)

class _Rng:

    def __init__(self, key):
        self._k = key

    def _next(self):
        self._k, sub = jax.random.split(self._k)
        return sub

    def normal(self, shape):
        return jax.random.normal(self._next(), shape, dtype=jnp.bfloat16)

    def randint(self, lo, hi, shape):
        return jax.random.randint(self._next(), shape, lo, hi, dtype=jnp.int32)

    def uniform(self, shape, lo=0.0, hi=1.0):
        return jax.random.uniform(self._next(), shape, jnp.bfloat16, lo, hi)

    def permutation(self, n):
        return jax.random.permutation(self._next(), n)
kernel_name = 'adaLN_cond__memory_aug_recurrent_mem_tr__moe_arch_mod__prompt'

def setup_inputs():
    _rng = _Rng(jax.random.key(int.from_bytes(__import__("os").urandom(4), "little")))
    _w = lambda a: (lambda t: t.astype(jnp.bfloat16) if jnp.issubdtype(t.dtype, jnp.floating) else t)(jnp.asarray(a))

    def _A_setup():
        B, S, Dm = (1, 2048, 1024)
        H, Dh = (32, 128)
        M, seg = (8, 32)
        seg = min(seg, S)
        S = S // seg * seg
        return {'x': _w((lambda *s: _rng.normal(s) * 0.05)(B, S, Dm)), 'mem0': _w((lambda *s: _rng.normal(s) * 0.05)(B, M, Dm)), 'Wq': _w((lambda *s: _rng.normal(s) * 0.05)(Dm, H, Dh) * Dm ** (-0.5)), 'Wk': _w((lambda *s: _rng.normal(s) * 0.05)(Dm, H, Dh) * Dm ** (-0.5)), 'Wv': _w((lambda *s: _rng.normal(s) * 0.05)(Dm, H, Dh) * Dm ** (-0.5)), 'Wo': _w((lambda *s: _rng.normal(s) * 0.05)(H, Dh, Dm) * (H * Dh) ** (-0.5)), 'seg_len': seg}
    _A_in = _A_setup()

    def _B_setup():
        B, S, D, F, C = (1, 2048, 1024, 3584, 2)
        return {'x': _w((lambda *s: _rng.normal(s) * 0.05)(B, S, D)), 'w_r': _w((lambda *s: _rng.normal(s) * 0.05)(D)), 'w_gate': _w((lambda *s: _rng.normal(s) * 0.05)(D, F)), 'w_up': _w((lambda *s: _rng.normal(s) * 0.05)(D, F)), 'w_down': _w((lambda *s: _rng.normal(s) * 0.05)(F, D))}
    _B_in = _B_setup()
    return {'A_x': _A_in['x'], 'A_mem0': _A_in['mem0'], 'A_Wq': _A_in['Wq'], 'A_Wk': _A_in['Wk'], 'A_Wv': _A_in['Wv'], 'A_Wo': _A_in['Wo'], 'A_seg_len': _A_in['seg_len'], 'B_x': _B_in['x'], 'B_w_r': _B_in['w_r'], 'B_w_gate': _B_in['w_gate'], 'B_w_up': _B_in['w_up'], 'B_w_down': _B_in['w_down'], 'c': _w((lambda *s: _rng.normal(s) * 0.05)(1, 1024)), 'w_mod': _w((lambda *s: _rng.normal(s) * 0.05)(1024, 6 * 1024) * 1024 ** (-0.5))}

def reference(A_x, A_mem0, A_Wq, A_Wk, A_Wv, A_Wo, A_seg_len, B_x, B_w_r, B_w_gate, B_w_up, B_w_down, c, w_mod):

    def _A_ref(x, mem0, Wq, Wk, Wv, Wo, seg_len):
        B, S, Dm = x.shape
        H, Dh = (Wq.shape[1], Wq.shape[2])
        M = mem0.shape[1]
        scale = Dh ** (-0.5)
        n_seg = S // seg_len
        L = M + seg_len
        idx = jnp.arange(L)
        mask = (idx[:, None] < M) | (idx[:, None] >= idx[None, :])
        mem = mem0
        outs = []
        for s in range(n_seg):
            xs = x[:, s * seg_len:(s + 1) * seg_len, :].copy()
            h = jnp.concatenate([mem, xs], axis=1)
            q = jnp.einsum('btd,dhe->bhte', h, Wq)
            k = jnp.einsum('btd,dhe->bhte', h, Wk)
            v = jnp.einsum('btd,dhe->bhte', h, Wv)
            scores = jnp.einsum('bhqe,bhke->bhqk', q, k) * scale
            scores = jnp.where(mask[None, None], scores, -1000000000.0)
            p = _softmax(scores, axis=-1)
            o = jnp.einsum('bhqk,bhke->bhqe', p, v)
            o = jnp.einsum('bhte,hed->btd', o, Wo)
            mem = o[:, :M, :].copy()
            outs.append(o[:, M:, :])
        return jnp.concatenate(outs, axis=1)

    def _B_ref(x, w_r, w_gate, w_up, w_down):
        B, S, D = x.shape
        C = 2
        r = x @ w_r
        idx = jnp.argsort(-r, axis=-1)[:, :C]
        idx_e = jnp.repeat(idx.reshape(B, C, 1), D, axis=2)
        x_sel = jnp.take_along_axis(x, idx_e, axis=1)
        g = _silu(x_sel @ w_gate)
        u = x_sel @ w_up
        y = g * u @ w_down
        r_sel = _sigmoid(jnp.take_along_axis(r, idx, axis=1))
        y = y * r_sel.reshape(B, C, 1)
        b_off = (jnp.arange(B) * S).reshape(B, 1)
        flat_idx = (idx + b_off).reshape(B * C)
        zero = (x * 0.0).reshape(B * S, D)
        upd = _scatter_add(zero, flat_idx, y.reshape(B * C, D), axis=0)
        return x + upd.reshape(B, S, D)
    x = A_x
    mod = (_silu(c) @ w_mod).reshape(c.shape[0], 6, 1, -1)
    sa, ca, ga, sb, cb, gb = (mod[:, 0].copy(), mod[:, 1].copy(), mod[:, 2].copy(), mod[:, 3].copy(), mod[:, 4].copy(), mod[:, 5].copy())
    h = _layernorm(x, axis=-1) * (1 + ca) + sa
    x = x + ga * _A_ref(h, A_mem0, A_Wq, A_Wk, A_Wv, A_Wo, A_seg_len)
    h = _layernorm(x, axis=-1) * (1 + cb) + sb
    x = x + gb * _B_ref(h, B_w_r, B_w_gate, B_w_up, B_w_down)
    return x
```

```python
import functools
import jax, jax.numpy as jnp, numpy as np
from jax import lax
from jax.experimental import pallas as pl
from jax.experimental.pallas import tpu as pltpu

S, D, H, DH, MM, SEG = 2048, 1024, 32, 128, 8, 32
L = MM + SEG
NSEG = S // SEG
F = 3584
HD = H * DH
BF = jnp.bfloat16
F32 = jnp.float32
U32 = jnp.uint32
EPS = 1e-5
NP = H // 2
FT = F // 128


def _ln(x):
    m = jnp.mean(x, axis=-1, keepdims=True)
    xc = x - m
    v = jnp.mean(xc * xc, axis=-1, keepdims=True)
    return xc * lax.rsqrt(v + EPS)


def _bf(u):
    return pltpu.bitcast(u, BF)


def _silu(x):
    return x * jax.nn.sigmoid(x)


def kernel(x_hbm, mem_ref, wq_hbm, wk_hbm, wv_hbm, wo_hbm, wr_ref, wg_hbm, wu_hbm, wd_hbm, c_ref, wm_hbm,
           o_hbm,
           xs, hbuf, hb, wqkv, wo, wma, wmb, raw, ring, mem, rs, outs, mods, aout, sems, wsem,
           *, G, LA, LB, TAILPOS, R, RING, LAG, UNROLL, DIST, PU, WS, N1P):
    NG = H // G
    GW = G * DH
    N1 = N1P or (S - R - 24 * (NSEG - 1)) // 8
    SEM_WMA, SEM_X0, SEM_X1, SEM_WO, SEM_WMB, SEM_FFN, SEM_OUT, SEM_FIX0, SEM_FIX1 = range(9)

    cp_wma = pltpu.make_async_copy(wm_hbm.at[:, pl.ds(0, 2 * D)], wma.bitcast(BF), sems.at[SEM_WMA]); cp_wma.start()
    cp_x0 = pltpu.make_async_copy(x_hbm.at[pl.ds(0, R)], xs.at[pl.ds(0, R)], sems.at[SEM_X0]); cp_x0.start()
    w32 = [w.bitcast(U32) for w in (wq_hbm, wk_hbm, wv_hbm)]

    def wcopy(w, p, par):
        return pltpu.make_async_copy(w32[w].at[:, par, p, :], raw.at[w * 2 * NP + 2 * p + par], wsem.at[w, p])
    XC = 144; NX = (S - R) // XC; assert NX * XC == S - R

    def xcopy(p):
        r0 = pl.multiple_of(R + p * XC, 16)
        return pltpu.make_async_copy(x_hbm.at[pl.ds(r0, XC)], xs.at[pl.ds(r0, XC)], sems.at[SEM_X1])

    def wocopy(p):
        r0 = pl.multiple_of(p * 256, 256)
        return pltpu.make_async_copy(wo_hbm.at[pl.ds(r0, 256)], wo.bitcast(BF).at[pl.ds(r0, 256)], sems.at[SEM_WO])
    for p in range(DIST):
        for par in range(2):
            wcopy(0, p, par).start()
    cp_wmb = pltpu.make_async_copy(wm_hbm.at[:, pl.ds(2 * D, 4 * D)], wmb.bitcast(BF), sems.at[SEM_WMB])

    def ffn_copies():
        cps = []
        for j in range(FT):
            cps.append(pltpu.make_async_copy(wg_hbm.at[:, pl.ds(j * 128, 128)], raw.at[j].bitcast(BF), sems.at[SEM_FFN]))
            cps.append(pltpu.make_async_copy(wu_hbm.at[:, pl.ds(j * 128, 128)], raw.at[FT + j].bitcast(BF), sems.at[SEM_FFN]))
        for kc in range(4):
            nr = min(D, F - kc * D)
            for n in range(D // 128):
                cps.append(pltpu.make_async_copy(wd_hbm.at[pl.ds(kc * D, nr), pl.ds(n * 128, 128)],
                                                 raw.at[2 * FT + kc * 8 + n, pl.ds(0, nr // 2)].bitcast(BF), sems.at[SEM_FFN]))
        return cps

    def out_copy(j):
        r0 = pl.multiple_of(j * 256, 256)
        return pltpu.make_async_copy(outs.at[pl.ds(r0, 256)], o_hbm.at[pl.ds(r0, 256)], sems.at[SEM_OUT])

    aout[...] = jnp.zeros_like(aout)
    mods[...] = jnp.zeros_like(mods)
    xs[S:S + SEG, :] = jnp.zeros((SEG, D), BF)
    hbuf[S:S + SEG, :] = jnp.zeros((SEG, D), F32)
    mem[...] = mem_ref[...].astype(F32)
    sc = jnp.broadcast_to(_silu(c_ref[...].astype(F32)), (8, D))
    cp_x0.wait()
    hbuf[0:R, :] = _ln(xs[0:R, :].astype(F32))
    if True:
        cp_wma.wait()
    for j in range(2):
        mods[8 * j:8 * j + 8, :] = jnp.dot(sc, _bf(wma[:, j * D:(j + 1) * D]), preferred_element_type=F32)

    hbuf[0:R, :] = hbuf[0:R, :] * (1.0 + mods[8:9, :]) + mods[0:1, :]
    hb[...] = hbuf[0:R, :].astype(BF)

    def pro(w):
        def body(p, _):
            for par in range(2):
                wcopy(w, p, par).wait()

            @pl.when(p + DIST < NP)
            def _():
                for par in range(2):
                    wcopy(w, p + DIST, par).start()
            if w < 2:
                @pl.when(p + DIST >= NP)
                def _():
                    for par in range(2):
                        wcopy(w + 1, p + DIST - NP, par).start()
            if w == 0:
                @pl.when(p < NX)
                def _():
                    xcopy(p).start()
            else:
                @pl.when(p % 2 == 0)
                def _():
                    wocopy((w - 1) * (NP // 2) + p // 2).start()
            if w == 1:
                r0 = pl.multiple_of(R + jnp.minimum(p, NX - 1) * XC, 16)
                hbuf[pl.ds(r0, XC), :] = _ln(xs[pl.ds(r0, XC), :].astype(F32)) * (1.0 + mods[8:9, :]) + mods[0:1, :]
            a = raw[w * 2 * NP + 2 * p]
            b = raw[w * 2 * NP + 2 * p + 1]
            lo = (a & jnp.uint32(0xffff)) | (b << 16)
            hi = (a >> 16) | (b & jnp.uint32(0xffff0000))
            for t, u in enumerate((lo, hi)):
                c0 = pl.multiple_of(p * 256 + t * 128, 128)
                wqkv[w, :, pl.ds(c0, 128)] = u
                ring[w, 0:R, pl.ds(c0, 128)] = jnp.dot(hb[...], _bf(u), preferred_element_type=F32)
            return 0
        lax.fori_loop(0, NP, body, 0, unroll=PU)
    if True:
        pro(0)
    for p in range(NX):
        xcopy(p).wait()
    if True:
        pro(1)
    if True:
        pro(2)
    cp_wmb.start()
    if True:
      for p in range(NP):
        wocopy(p).wait()

    scale = DH ** -0.5
    qi = lax.broadcasted_iota(jnp.int32, (L, L), 0)
    kj = lax.broadcasted_iota(jnp.int32, (L, L), 1)
    mask = (qi < MM) | (qi >= kj)

    def tail(t, slot):
        r0 = pl.multiple_of(t * SEG, SEG)
        x1 = xs[pl.ds(r0, SEG), :].astype(F32) + mods[16:17, :] * aout[slot]
        x1b = x1.astype(BF)
        xs[pl.ds(r0, SEG), :] = x1b
        h2 = _ln(x1b.astype(F32)) * (1.0 + mods[32:33, :]) + mods[24:25, :]
        r = jnp.sum(h2 * wr_ref[...].astype(F32), axis=-1, keepdims=True)
        rs[pl.ds(r0, SEG), :] = jnp.broadcast_to(r, (SEG, 128))
        outs[pl.ds(r0, SEG), :] = (x1 + mods[40:41, :] * h2).astype(BF)

    def qk(q, k):
        ps = []
        for h in range(G):
            sl = slice(h * DH, (h + 1) * DH)
            sc_ = lax.dot_general(q[:, sl] * scale, k[:, sl], (((1,), (1,)), ((), ())), preferred_element_type=F32)
            sc_ = jnp.where(mask, sc_, -1e9)
            m = jnp.max(sc_, axis=-1, keepdims=True)
            e = jnp.exp(sc_ - m)
            ps.append(e * (1.0 / jnp.sum(e, axis=-1, keepdims=True)))
        return ps

    def pv(ps, v):
        os_ = [jnp.dot(ps[h], v[:, h * DH:(h + 1) * DH], preferred_element_type=F32) for h in range(G)]
        return jnp.concatenate(os_, axis=1)

    def step(s, nx, row0):
        @pl.when(s == LAG)
        def _():
            cp_wmb.wait()
            for j in range(4):
                mods[16 + 8 * j:24 + 8 * j, :] = jnp.dot(sc, _bf(wmb[:, j * D:(j + 1) * D]), preferred_element_type=F32)
            for cp in ffn_copies():
                cp.start()

        @pl.when((s >= 8 + LAG) & ((s - LAG) % 8 == 0))
        def _():
            out_copy((s - LAG) // 8 - 1).start()

        row0 = pl.multiple_of(row0, 8)
        lhs = jnp.concatenate([mem[...], hbuf[pl.ds(row0, 8 * nx), :]], axis=0)
        wpos = [pl.multiple_of(((row0 // 8 + i) % (RING // 8)) * 8, 8) for i in range(nx)]
        rpos = pl.multiple_of((s % (RING // SEG)) * SEG, SEG)

        def projw(w, g):
            cs = slice(g * GW, (g + 1) * GW)
            old = ring[w, pl.ds(rpos, SEG), cs]
            y = jnp.dot(lhs, _bf(wqkv[w, :, cs]), preferred_element_type=F32)
            for i in range(nx):
                ring[w, pl.ds(wpos[i], 8), cs] = y[8 + 8 * i:16 + 8 * i]
            return jnp.concatenate([y[0:MM], old], axis=0)

        QK, P, V, O = {}, {}, {}, {}
        for g in range(NG):
            QK[g] = (projw(0, g), projw(1, g).astype(BF))
            if g == TAILPOS:
                tail(jnp.where(s >= LAG, s - LAG, NSEG), (s + 1) % (LAG + 1))
            if g >= LA:
                P[g - LA] = qk(*QK.pop(g - LA))
        st = dict(out=None, done=0)

        def wo_part(g1):
            g0 = st["done"]
            o = jnp.concatenate([O.pop(g) for g in range(g0, g1)], axis=1)
            y = jnp.dot(o, _bf(wo[g0 * GW // 2:g1 * GW // 2, :]), preferred_element_type=F32)
            st["out"] = y if st["out"] is None else st["out"] + y
            st["done"] = g1
        sched = dict(WS)
        for g in range(NG + LB + 1):
            if g < NG:
                V[g] = projw(2, g).astype(BF)
            if g < LA:
                P[NG - LA + g] = qk(*QK.pop(NG - LA + g))
            if g in sched:
                wo_part(sched[g])
            if LB <= g < NG + LB:
                O[g - LB] = pv(P.pop(g - LB), V.pop(g - LB))
        assert st["done"] == NG
        out = st["out"]
        mem[...] = out[0:MM]
        aout[s % (LAG + 1)] = out[MM:L]
        return 0

    if True:
      lax.fori_loop(0, N1, lambda s, _: step(s, 4, R + 32 * s), 0, unroll=UNROLL)
    if True:
      lax.fori_loop(N1, NSEG, lambda s, _: step(s, 3, R + 32 * N1 + 24 * (s - N1)), 0, unroll=UNROLL)
    for t in range(NSEG - LAG, NSEG):
        tail(t, t % (LAG + 1))
    out_copy(7).start()

    r = rs[0:S, :].astype(BF).astype(F32)
    ridx = lax.broadcasted_iota(jnp.int32, (S, 128), 0)
    m1 = jnp.max(r)
    i1 = jnp.min(jnp.where(r == m1, ridx, S))
    r2 = jnp.where(ridx == i1, -jnp.inf, r)
    m2 = jnp.max(r2)
    i2 = jnp.min(jnp.where((r2 == m2) & (ridx != i1), ridx, S))
    i1 = jnp.minimum(i1, S - 1)
    i2 = jnp.minimum(i2, S - 1)
    ri16 = lax.broadcasted_iota(jnp.int32, (16, D), 0)
    rowi = lax.broadcasted_iota(jnp.int32, (8, D), 0)

    def getrow(ii):
        b0 = pl.multiple_of((ii // 16) * 16, 16)
        blk = xs[pl.ds(b0, 16), :].astype(F32)
        return jnp.sum(jnp.where(ri16 == ii - b0, blk, 0.0), axis=0, keepdims=True)
    xsel = jnp.where(rowi == 0, getrow(i1), getrow(i2))
    h2 = _ln(xsel) * (1.0 + mods[32:33, :]) + mods[24:25, :]
    for cp in ffn_copies():
        cp.wait()
    h2b = h2.astype(BF).astype(F32)
    acts = []
    for j in range(FT):
        gg = jnp.dot(h2b, _bf(raw[j]), preferred_element_type=F32)
        uu = jnp.dot(h2b, _bf(raw[FT + j]), preferred_element_type=F32)
        acts.append(_silu(gg) * uu)
    ys = []
    for n in range(D // 128):
        y = None
        for kc in range(4):
            nr = min(D, F - kc * D)
            a = jnp.concatenate(acts[kc * 8:kc * 8 + nr // 128], axis=1)
            t = jnp.dot(a, _bf(raw[2 * FT + kc * 8 + n, 0:nr // 2]), preferred_element_type=F32)
            y = t if y is None else y + t
        ys.append(y)
    y = jnp.concatenate(ys, axis=1)
    rsel = jnp.where(rowi[:, 0:1] == 0, m1, m2)
    osel = xsel + mods[40:41, :] * (h2 + y * jax.nn.sigmoid(rsel))
    for j in range(8):
        out_copy(j).wait()
    bs = []
    for j, ii in enumerate((i1, i2)):
        b0 = pl.multiple_of((ii // 16) * 16, 16)
        blk = outs[pl.ds(b0, 16), :].astype(F32)
        outs[pl.ds(b0, 16), :] = jnp.where(ri16 == ii - b0, osel[j:j + 1, :], blk).astype(BF)
        bs.append(b0)
    fix = [pltpu.make_async_copy(outs.at[pl.ds(bs[j], 16)], o_hbm.at[pl.ds(bs[j], 16)], sems.at[SEM_FIX0 + j]) for j in range(2)]
    fix[0].start()

    @pl.when(bs[0] != bs[1])
    def _():
        fix[1].start()
        fix[1].wait()
    fix[0].wait()


def build(G=4, LA=1, LB=1, TAILPOS=1, R=320, RING=352, LAG=3, UNROLL=1, DIST=6, PU=1, WS=((6,3),(8,6),(9,8)), N1P=0):
    def f(A_x, A_mem0, A_Wq, A_Wk, A_Wv, A_Wo, A_seg_len, B_x, B_w_r, B_w_gate, B_w_up, B_w_down, c, w_mod):
        any_ = pl.BlockSpec(memory_space=pl.ANY)
        vm = pl.BlockSpec(memory_space=pltpu.VMEM)
        out = pl.pallas_call(
            functools.partial(kernel, G=G, LA=LA, LB=LB, TAILPOS=TAILPOS, R=R, RING=RING, LAG=LAG, UNROLL=UNROLL, DIST=DIST, PU=PU, WS=WS, N1P=N1P),
            out_shape=jax.ShapeDtypeStruct((S, D), BF),
            in_specs=[any_, vm, any_, any_, any_, any_, vm, any_, any_, any_, vm, any_],
            out_specs=any_,
            scratch_shapes=[
                pltpu.VMEM((S + SEG, D), BF),
                pltpu.VMEM((S + SEG, D), F32),
                pltpu.VMEM((R, D), BF),
                pltpu.VMEM((3, D // 2, HD), U32),
                pltpu.VMEM((HD // 2, D), U32),
                pltpu.VMEM((D // 2, 2 * D), U32),
                pltpu.VMEM((D // 2, 4 * D), U32),
                pltpu.VMEM((6 * NP, 512, 128), U32),
                pltpu.VMEM((3, RING, HD), F32),
                pltpu.VMEM((MM, D), F32),
                pltpu.VMEM((S + SEG, 128), F32),
                pltpu.VMEM((S + SEG, D), BF),
                pltpu.VMEM((48, D), F32),
                pltpu.VMEM((LAG + 1, SEG, D), F32),
                pltpu.SemaphoreType.DMA((9,)),
                pltpu.SemaphoreType.DMA((3, NP)),
            ],
            compiler_params=pltpu.CompilerParams(vmem_limit_bytes=120 * 2**20),
        )(A_x.reshape(S, D), A_mem0.reshape(MM, D),
          A_Wq.reshape(512, 2, H, DH), A_Wk.reshape(512, 2, H, DH), A_Wv.reshape(512, 2, H, DH),
          A_Wo.reshape(HD, D), B_w_r.reshape(1, D), B_w_gate, B_w_up, B_w_down, c, w_mod)
        return out.reshape(1, S, D)
    return jax.jit(f, static_argnames=("A_seg_len",))


_impl = build()


def pallas_adaLN_cond__memory_aug_recurrent_mem_tr__moe_arch_mod__prompt_kernel(
        A_x, A_mem0, A_Wq, A_Wk, A_Wv, A_Wo, A_seg_len, B_x, B_w_r, B_w_gate, B_w_up, B_w_down, c, w_mod):
    return _impl(A_x, A_mem0, A_Wq, A_Wk, A_Wv, A_Wo, A_seg_len, B_x, B_w_r, B_w_gate, B_w_up, B_w_down, c, w_mod)
```

```python
import functools
import jax, jax.numpy as jnp, numpy as np
from jax import lax
from jax.experimental import pallas as pl
from jax.experimental.pallas import tpu as pltpu

S, D, H, DH, MM, SEG = 2048, 1024, 32, 128, 8, 32
L = MM + SEG
NSEG = S // SEG
F = 3584
HD = H * DH
BF = jnp.bfloat16
F32 = jnp.float32
U32 = jnp.uint32
EPS = 1e-5
NP = H // 2
FT = F // 128


def _ln(x):
    m = jnp.mean(x, axis=-1, keepdims=True)
    xc = x - m
    v = jnp.mean(xc * xc, axis=-1, keepdims=True)
    return xc * lax.rsqrt(v + EPS)


def _bf(u):
    return pltpu.bitcast(u, BF)


def _silu(x):
    return x * jax.nn.sigmoid(x)


def kernel(x_hbm, mem_ref, wq_hbm, wk_hbm, wv_hbm, wo_hbm, wr_ref, wg_hbm, wu_hbm, wd_hbm, c_ref, wm_hbm,
           o_hbm,
           xs, hbuf, hb, wqkv, wo, wma, wmb, raw, ring, mem, rs, outs, mods, aout, sems, wsem,
           *, G, LA, LB, TAILPOS, R, RING, LAG, UNROLL, DIST, PU, WS, N1P, D0):
    NG = H // G
    GW = G * DH
    N1 = N1P or (S - R - 24 * (NSEG - 1)) // 8
    SEM_WMA, SEM_X0, SEM_X1, SEM_WO, SEM_WMB, SEM_FFN, SEM_OUT, SEM_FIX0, SEM_FIX1 = range(9)

    cp_x0 = pltpu.make_async_copy(x_hbm.at[pl.ds(0, R)], xs.at[pl.ds(0, R)], sems.at[SEM_X0]); cp_x0.start()
    cp_wma = pltpu.make_async_copy(wm_hbm.at[:, pl.ds(0, 2 * D)], wma.bitcast(BF), sems.at[SEM_WMA]); cp_wma.start()
    w32 = [w.bitcast(U32) for w in (wq_hbm, wk_hbm, wv_hbm)]

    def wcopy(w, p, par):
        return pltpu.make_async_copy(w32[w].at[:, par, p, :], raw.at[w * 2 * NP + 2 * p + par], wsem.at[w, p])
    XC = 144; NX = (S - R) // XC; assert NX * XC == S - R

    def xcopy(p):
        r0 = pl.multiple_of(R + p * XC, 16)
        return pltpu.make_async_copy(x_hbm.at[pl.ds(r0, XC)], xs.at[pl.ds(r0, XC)], sems.at[SEM_X1])

    def wocopy(p):
        r0 = pl.multiple_of(p * 256, 256)
        return pltpu.make_async_copy(wo_hbm.at[pl.ds(r0, 256)], wo.bitcast(BF).at[pl.ds(r0, 256)], sems.at[SEM_WO])
    for p in range(D0):
        for par in range(2):
            wcopy(0, p, par).start()
    cp_wmb = pltpu.make_async_copy(wm_hbm.at[:, pl.ds(2 * D, 4 * D)], wmb.bitcast(BF), sems.at[SEM_WMB])

    def ffn_copies():
        cps = []
        for j in range(FT):
            cps.append(pltpu.make_async_copy(wg_hbm.at[:, pl.ds(j * 128, 128)], raw.at[j].bitcast(BF), sems.at[SEM_FFN]))
            cps.append(pltpu.make_async_copy(wu_hbm.at[:, pl.ds(j * 128, 128)], raw.at[FT + j].bitcast(BF), sems.at[SEM_FFN]))
        for kc in range(4):
            nr = min(D, F - kc * D)
            for n in range(D // 128):
                cps.append(pltpu.make_async_copy(wd_hbm.at[pl.ds(kc * D, nr), pl.ds(n * 128, 128)],
                                                 raw.at[2 * FT + kc * 8 + n, pl.ds(0, nr // 2)].bitcast(BF), sems.at[SEM_FFN]))
        return cps

    def out_copy(j):
        r0 = pl.multiple_of(j * 256, 256)
        return pltpu.make_async_copy(outs.at[pl.ds(r0, 256)], o_hbm.at[pl.ds(r0, 256)], sems.at[SEM_OUT])

    aout[...] = jnp.zeros_like(aout)
    for j in range(2):
        rs[2 * j] = jnp.full((SEG, 128), -jnp.inf, F32)
        rs[2 * j + 1] = jnp.full((SEG, 128), float(S), F32)
    mods[...] = jnp.zeros_like(mods)
    xs[S:S + SEG, :] = jnp.zeros((SEG, D), BF)
    hbuf[S:S + SEG, :] = jnp.zeros((SEG, D), F32)
    mem[...] = mem_ref[...].astype(F32)
    sc = jnp.broadcast_to(_silu(c_ref[...].astype(F32)), (8, D))
    cp_x0.wait()
    hbuf[0:R, :] = _ln(xs[0:R, :].astype(F32))
    if True:
        cp_wma.wait()
    for p in range(D0, DIST):
        for par in range(2):
            wcopy(0, p, par).start()
    for j in range(2):
        mods[8 * j:8 * j + 8, :] = jnp.dot(sc, _bf(wma[:, j * D:(j + 1) * D]), preferred_element_type=F32)

    hbuf[0:R, :] = hbuf[0:R, :] * (1.0 + mods[8:9, :]) + mods[0:1, :]
    hb[...] = hbuf[0:R, :].astype(BF)

    def pro(w):
        def body(p, _):
            for par in range(2):
                wcopy(w, p, par).wait()

            @pl.when(p + DIST < NP)
            def _():
                for par in range(2):
                    wcopy(w, p + DIST, par).start()
            if w < 2:
                @pl.when(p + DIST >= NP)
                def _():
                    for par in range(2):
                        wcopy(w + 1, p + DIST - NP, par).start()
            if w == 0:
                @pl.when(p < NX)
                def _():
                    xcopy(p).start()
            else:
                @pl.when(p % 2 == 0)
                def _():
                    wocopy((w - 1) * (NP // 2) + p // 2).start()
            if w == 1:
                r0 = pl.multiple_of(R + jnp.minimum(p, NX - 1) * XC, 16)
                hbuf[pl.ds(r0, XC), :] = _ln(xs[pl.ds(r0, XC), :].astype(F32)) * (1.0 + mods[8:9, :]) + mods[0:1, :]
            a = raw[w * 2 * NP + 2 * p]
            b = raw[w * 2 * NP + 2 * p + 1]
            lo = (a & jnp.uint32(0xffff)) | (b << 16)
            hi = (a >> 16) | (b & jnp.uint32(0xffff0000))
            for t, u in enumerate((lo, hi)):
                c0 = pl.multiple_of(p * 256 + t * 128, 128)
                wqkv[w, :, pl.ds(c0, 128)] = u
                ring[w, 0:R, pl.ds(c0, 128)] = jnp.dot(hb[...], _bf(u), preferred_element_type=F32)
            return 0
        lax.fori_loop(0, NP, body, 0, unroll=PU)
    if True:
        pro(0)
    for p in range(NX):
        xcopy(p).wait()
    if True:
        pro(1)
    if True:
        pro(2)
    cp_wmb.start()
    if True:
      for p in range(NP):
        wocopy(p).wait()

    scale = DH ** -0.5
    qi = lax.broadcasted_iota(jnp.int32, (L, L), 0)
    kj = lax.broadcasted_iota(jnp.int32, (L, L), 1)
    mask = (qi < MM) | (qi >= kj)

    def tail(t, slot):
        r0 = pl.multiple_of(t * SEG, SEG)
        x1 = xs[pl.ds(r0, SEG), :].astype(F32) + mods[16:17, :] * aout[slot]
        x1b = x1.astype(BF)
        xs[pl.ds(r0, SEG), :] = x1b
        h2 = _ln(x1b.astype(F32)) * (1.0 + mods[32:33, :]) + mods[24:25, :]
        r = jnp.sum(h2 * wr_ref[...].astype(F32), axis=-1, keepdims=True)
        r = jnp.broadcast_to(r.astype(BF).astype(F32), (SEG, 128))
        r = jnp.where(t < NSEG, r, -jnp.inf)
        ix = (t * SEG + lax.broadcasted_iota(jnp.int32, (SEG, 128), 0)).astype(F32)
        b1, j1, b2, j2 = rs[0], rs[1], rs[2], rs[3]
        g1 = r > b1
        g2 = r > b2
        rs[0] = jnp.where(g1, r, b1)
        rs[1] = jnp.where(g1, ix, j1)
        rs[2] = jnp.where(g1, b1, jnp.where(g2, r, b2))
        rs[3] = jnp.where(g1, j1, jnp.where(g2, ix, j2))
        outs[pl.ds(r0, SEG), :] = (x1 + mods[40:41, :] * h2).astype(BF)

    def qk(q, k):
        ps = []
        for h in range(G):
            sl = slice(h * DH, (h + 1) * DH)
            sc_ = lax.dot_general(q[:, sl] * scale, k[:, sl], (((1,), (1,)), ((), ())), preferred_element_type=F32)
            sc_ = jnp.where(mask, sc_, -1e9)
            m = jnp.max(sc_, axis=-1, keepdims=True)
            e = jnp.exp(sc_ - m)
            ps.append(e * (1.0 / jnp.sum(e, axis=-1, keepdims=True)))
        return ps

    def pv(ps, v):
        os_ = [jnp.dot(ps[h], v[:, h * DH:(h + 1) * DH], preferred_element_type=F32) for h in range(G)]
        return jnp.concatenate(os_, axis=1)

    def mods2():
            cp_wmb.wait()
            for j in range(4):
                mods[16 + 8 * j:24 + 8 * j, :] = jnp.dot(sc, _bf(wmb[:, j * D:(j + 1) * D]), preferred_element_type=F32)
            for cp in ffn_copies():
                cp.start()

    def step(s, nx, row0):
        if nx == 4:
            pl.when(s == LAG)(mods2)

        @pl.when((s >= 8 + LAG) & ((s - LAG) % 8 == 0))
        def _():
            out_copy((s - LAG) // 8 - 1).start()

        row0 = pl.multiple_of(row0, 8)
        lhs = jnp.concatenate([mem[...], hbuf[pl.ds(row0, 8 * nx), :]], axis=0)
        wpos = [pl.multiple_of(((row0 // 8 + i) % (RING // 8)) * 8, 8) for i in range(nx)]
        rpos = pl.multiple_of((s % (RING // SEG)) * SEG, SEG)

        def projw(w, g):
            cs = slice(g * GW, (g + 1) * GW)
            old = ring[w, pl.ds(rpos, SEG), cs]
            y = jnp.dot(lhs, _bf(wqkv[w, :, cs]), preferred_element_type=F32)
            for i in range(nx):
                ring[w, pl.ds(wpos[i], 8), cs] = y[8 + 8 * i:16 + 8 * i]
            return jnp.concatenate([y[0:MM], old], axis=0)

        QK, P, V, O = {}, {}, {}, {}
        for g in range(NG):
            QK[g] = (projw(0, g), projw(1, g).astype(BF))
            if g == TAILPOS:
                tail(jnp.where(s >= LAG, s - LAG, NSEG), (s + 1) % (LAG + 1))
            if g >= LA:
                P[g - LA] = qk(*QK.pop(g - LA))
        st = dict(out=None, done=0)

        def wo_part(g1):
            g0 = st["done"]
            o = jnp.concatenate([O.pop(g) for g in range(g0, g1)], axis=1)
            y = jnp.dot(o, _bf(wo[g0 * GW // 2:g1 * GW // 2, :]), preferred_element_type=F32)
            st["out"] = y if st["out"] is None else st["out"] + y
            st["done"] = g1
        sched = dict(WS)
        for g in range(NG + LB + 1):
            if g < NG:
                V[g] = projw(2, g).astype(BF)
            if g < LA:
                P[NG - LA + g] = qk(*QK.pop(NG - LA + g))
            if g in sched:
                wo_part(sched[g])
            if LB <= g < NG + LB:
                O[g - LB] = pv(P.pop(g - LB), V.pop(g - LB))
        assert st["done"] == NG
        out = st["out"]
        mem[...] = out[0:MM]
        aout[s % (LAG + 1)] = out[MM:L]
        return 0

    if True:
      lax.fori_loop(0, N1, lambda s, _: step(s, 4, R + 32 * s), 0, unroll=UNROLL)
    if True:
      lax.fori_loop(N1, NSEG, lambda s, _: step(s, 3, R + 32 * N1 + 24 * (s - N1)), 0, unroll=UNROLL)
    for t in range(NSEG - LAG, NSEG):
        tail(t, t % (LAG + 1))
    out_copy(7).start()

    r = jnp.concatenate([rs[0], rs[2]], axis=0)
    ridx = jnp.concatenate([rs[1], rs[3]], axis=0).astype(jnp.int32)
    m1 = jnp.max(r)
    i1 = jnp.min(jnp.where(r == m1, ridx, S))
    r2 = jnp.where(ridx == i1, -jnp.inf, r)
    m2 = jnp.max(r2)
    i2 = jnp.min(jnp.where((r2 == m2) & (ridx != i1), ridx, S))
    i1 = jnp.minimum(i1, S - 1)
    i2 = jnp.minimum(i2, S - 1)
    ri16 = lax.broadcasted_iota(jnp.int32, (16, D), 0)
    rowi = lax.broadcasted_iota(jnp.int32, (8, D), 0)

    def getrow(ii):
        b0 = pl.multiple_of((ii // 16) * 16, 16)
        blk = xs[pl.ds(b0, 16), :].astype(F32)
        return jnp.sum(jnp.where(ri16 == ii - b0, blk, 0.0), axis=0, keepdims=True)
    xsel = jnp.where(rowi == 0, getrow(i1), getrow(i2))
    h2 = _ln(xsel) * (1.0 + mods[32:33, :]) + mods[24:25, :]
    for cp in ffn_copies():
        cp.wait()
    h2b = h2.astype(BF).astype(F32)
    acts = []
    for j in range(FT):
        gg = jnp.dot(h2b, _bf(raw[j]), preferred_element_type=F32)
        uu = jnp.dot(h2b, _bf(raw[FT + j]), preferred_element_type=F32)
        acts.append(_silu(gg) * uu)
    ys = []
    for n in range(D // 128):
        y = None
        for kc in range(4):
            nr = min(D, F - kc * D)
            a = jnp.concatenate(acts[kc * 8:kc * 8 + nr // 128], axis=1)
            t = jnp.dot(a, _bf(raw[2 * FT + kc * 8 + n, 0:nr // 2]), preferred_element_type=F32)
            y = t if y is None else y + t
        ys.append(y)
    y = jnp.concatenate(ys, axis=1)
    rsel = jnp.where(rowi[:, 0:1] == 0, m1, m2)
    osel = xsel + mods[40:41, :] * (h2 + y * jax.nn.sigmoid(rsel))
    for j in range(8):
        out_copy(j).wait()
    bs = []
    for j, ii in enumerate((i1, i2)):
        b0 = pl.multiple_of((ii // 16) * 16, 16)
        blk = outs[pl.ds(b0, 16), :].astype(F32)
        outs[pl.ds(b0, 16), :] = jnp.where(ri16 == ii - b0, osel[j:j + 1, :], blk).astype(BF)
        bs.append(b0)
    fix = [pltpu.make_async_copy(outs.at[pl.ds(bs[j], 16)], o_hbm.at[pl.ds(bs[j], 16)], sems.at[SEM_FIX0 + j]) for j in range(2)]
    fix[0].start()

    @pl.when(bs[0] != bs[1])
    def _():
        fix[1].start()
        fix[1].wait()
    fix[0].wait()


def build(G=2, LA=1, LB=1, TAILPOS=1, R=320, RING=352, LAG=2, UNROLL=1, DIST=6, PU=1, WS=((12,6),(16,12),(17,16)), N1P=0, D0=2):
    def f(A_x, A_mem0, A_Wq, A_Wk, A_Wv, A_Wo, A_seg_len, B_x, B_w_r, B_w_gate, B_w_up, B_w_down, c, w_mod):
        any_ = pl.BlockSpec(memory_space=pl.ANY)
        vm = pl.BlockSpec(memory_space=pltpu.VMEM)
        out = pl.pallas_call(
            functools.partial(kernel, G=G, LA=LA, LB=LB, TAILPOS=TAILPOS, R=R, RING=RING, LAG=LAG, UNROLL=UNROLL, DIST=DIST, PU=PU, WS=WS, N1P=N1P, D0=D0),
            out_shape=jax.ShapeDtypeStruct((S, D), BF),
            in_specs=[any_, vm, any_, any_, any_, any_, vm, any_, any_, any_, vm, any_],
            out_specs=any_,
            scratch_shapes=[
                pltpu.VMEM((S + SEG, D), BF),
                pltpu.VMEM((S + SEG, D), F32),
                pltpu.VMEM((R, D), BF),
                pltpu.VMEM((3, D // 2, HD), U32),
                pltpu.VMEM((HD // 2, D), U32),
                pltpu.VMEM((D // 2, 2 * D), U32),
                pltpu.VMEM((D // 2, 4 * D), U32),
                pltpu.VMEM((6 * NP, 512, 128), U32),
                pltpu.VMEM((3, RING, HD), F32),
                pltpu.VMEM((MM, D), F32),
                pltpu.VMEM((4, SEG, 128), F32),
                pltpu.VMEM((S + SEG, D), BF),
                pltpu.VMEM((48, D), F32),
                pltpu.VMEM((LAG + 1, SEG, D), F32),
                pltpu.SemaphoreType.DMA((9,)),
                pltpu.SemaphoreType.DMA((3, NP)),
            ],
            compiler_params=pltpu.CompilerParams(vmem_limit_bytes=120 * 2**20),
        )(A_x.reshape(S, D), A_mem0.reshape(MM, D),
          A_Wq.reshape(512, 2, H, DH), A_Wk.reshape(512, 2, H, DH), A_Wv.reshape(512, 2, H, DH),
          A_Wo.reshape(HD, D), B_w_r.reshape(1, D), B_w_gate, B_w_up, B_w_down, c, w_mod)
        return out.reshape(1, S, D)
    return jax.jit(f, static_argnames=("A_seg_len",))


_impl = build()


def pallas_adaLN_cond__memory_aug_recurrent_mem_tr__moe_arch_mod__prompt_kernel(
        A_x, A_mem0, A_Wq, A_Wk, A_Wv, A_Wo, A_seg_len, B_x, B_w_r, B_w_gate, B_w_up, B_w_down, c, w_mod):
    return _impl(A_x, A_mem0, A_Wq, A_Wk, A_Wv, A_Wo, A_seg_len, B_x, B_w_r, B_w_gate, B_w_up, B_w_down, c, w_mod)
```
